```python
import os as _os
_os.environ.setdefault("JAX_PLATFORMS", "cpu")
import jax
import jax.numpy as jnp

def _softmax(x, axis=-1):
    return jax.nn.softmax(x, axis=axis)
def _gelu(x):
    return jax.nn.gelu(x, approximate=True)
def _silu(x):
    return jax.nn.silu(x)
def _sigmoid(x):
    return jax.nn.sigmoid(x)
def _layernorm(x, axis=-1, eps=1e-5):
    m = jnp.mean(x, axis=axis, keepdims=True)
    v = jnp.var(x, axis=axis, keepdims=True)
    return (x - m) / jnp.sqrt(v + eps)
def _scatter_add(tgt, idx, src, axis=0):
    return tgt.at[idx].add(src)
def _segment_sum(src, seg, n):
    return jax.ops.segment_sum(src, seg, n)
class _Rng:
    def __init__(self, key):
        self._k = key
    def _next(self):
        self._k, sub = jax.random.split(self._k)
        return sub
    def normal(self, shape):
        return jax.random.normal(self._next(), shape, dtype=jnp.bfloat16)
    def randint(self, lo, hi, shape):
        return jax.random.randint(self._next(), shape, lo, hi, dtype=jnp.int32)
    def uniform(self, shape, lo=0.0, hi=1.0):
        return jax.random.uniform(self._next(), shape, jnp.bfloat16, lo, hi)
    def permutation(self, n):
        return jax.random.permutation(self._next(), n)


kernel_name = 'standalone__gqa_block_cached__near_ridge'

def setup_inputs():
    _rng = _Rng(jax.random.key(int.from_bytes(__import__("os").urandom(4), "little")))
    _w = (lambda a: (lambda t: t.astype(jnp.bfloat16) if jnp.issubdtype(t.dtype, jnp.floating) else t)(jnp.asarray(a)))
    B, Sq, D = 16, 128, 576
    Hq, Hkv, Sk, Dh = 32, 16, 1024, 128
    assert Hq % Hkv == 0, (Hq, Hkv)
    return {
        "x": _w((lambda *s: _rng.normal(s) * 0.8)(B, Sq, D)),
        "k_cache": _w((lambda *s: _rng.normal(s) * 0.8)(B, Hkv, Sk, Dh)),
        "v_cache": _w((lambda *s: _rng.normal(s) * 0.05)(B, Hkv, Sk, Dh)),
        "wq": _w((lambda *s: _rng.normal(s) * 0.8)(D, Hq * Dh) * (D ** -0.5)),
        "wo": _w((lambda *s: _rng.normal(s) * 0.05)(Hq * Dh, D) * ((Hq * Dh) ** -0.5)),
    }

def reference(x, k_cache, v_cache, wq, wo):
    B, Sq, D = x.shape
    Hq, Dh = 32, 128
    Hkv = k_cache.shape[1]
    rep = Hq // Hkv
    q = (lambda x, *d: x.transpose(*d))((x @ wq).reshape(B, Sq, Hq, Dh), 0, 2, 1, 3)
    k = jnp.repeat(k_cache, rep, axis=1)
    v = jnp.repeat(v_cache, rep, axis=1)
    scores = jnp.einsum("bhqd,bhkd->bhqk", q, k) * (Dh ** -0.5)
    p = _softmax(scores, axis=-1)
    o = jnp.einsum("bhqk,bhkd->bhqd", p, v)
    return (lambda x, *d: x.transpose(*d))(o, 0, 2, 1, 3).reshape(B, Sq, Hq * Dh) @ wo
```

```python
import functools
import math

import jax
import jax.numpy as jnp
import jax.experimental.pallas as pl
import jax.experimental.pallas.tpu as pltpu


HB = 4
BB = 2


def _kernel(xt_ref, k_ref, v_ref, wq_hbm, wot_hbm, o_ref,
            wq_ref, wot_ref, sem, acc_ref, x_ref, q_s, oc_s, s0, s1, p0, p1, l0, l1,
            *, rep, dh, hb, bb, ng):
    i = pl.program_id(0)
    j = pl.program_id(1)
    nj = pl.num_programs(1)
    scale = dh ** -0.5 * math.log2(math.e)
    sq = xt_ref.shape[2]
    w = rep * dh
    gw = hb * w
    n = hb * bb
    nt = (((1,), (1,)), ((), ()))
    sbuf, pbuf, lbuf = (s0, s1), (p0, p1), (l0, l1)

    def w_copy(which, g):
        src, dst = ((wq_hbm, wq_ref), (wot_hbm, wot_ref))[which]
        return pltpu.make_async_copy(src.at[:, pl.ds(g * gw, gw)], dst.at[g], sem.at[which, g])

    @pl.when(jnp.logical_and(i == 0, j == 0))
    def _():
        for g in range(ng):
            w_copy(0, g).start()
            w_copy(1, g).start()

    @pl.when(j == 0)
    def _():
        acc_ref[...] = jnp.zeros_like(acc_ref)
        for b in range(bb):
            x_ref[b * sq:(b + 1) * sq, :] = xt_ref[b].astype(jnp.float32).T.astype(jnp.bfloat16)

    @pl.when(i == 0)
    def _():
        w_copy(0, j).wait()
        w_copy(1, j).wait()

    q = jnp.dot(x_ref[...], wq_ref[j], preferred_element_type=jnp.float32)
    q = (q * scale).astype(jnp.bfloat16)
    for h in range(hb):
        for b in range(bb):
            for r in range(rep):
                q_s[h * bb + b, r * sq:(r + 1) * sq, :] = q[b * sq:(b + 1) * sq,
                                                            (h * rep + r) * dh:(h * rep + r + 1) * dh]

    def stage_a(u, par):
        sbuf[par][...] = jax.lax.dot_general(q_s[u], k_ref[u % bb, u // bb], nt,
                                             preferred_element_type=jnp.float32)

    def stage_b(par):
        s = sbuf[par][...]
        m = jnp.max(s, axis=-1, keepdims=True)
        p = jnp.exp2(s - m)
        lbuf[par][...] = jnp.sum(p, axis=-1, keepdims=True)
        pbuf[par][...] = p.astype(jnp.bfloat16)

    def stage_c(u, par):
        o = jnp.dot(pbuf[par][...], v_ref[u % bb, u // bb], preferred_element_type=jnp.float32)
        o = (o / lbuf[par][...]).astype(jnp.bfloat16)
        b, h = u % bb, u // bb
        for r in range(rep):
            oc_s[h * rep + r, pl.ds(pl.multiple_of(b * sq, sq), sq), :] = o[r * sq:(r + 1) * sq]

    def pair(e, first=False, last=False):
        if not first:
            stage_c(e - 1, 1)
        stage_a(e + 1, 1)
        stage_b(0)
        if not last:
            stage_a(e + 2, 0)
        stage_b(1)
        stage_c(e, 0)

    stage_a(0, 0)
    pair(0, first=True)

    def body(t, carry):
        pair(2 * t)
        return carry

    jax.lax.fori_loop(1, n // 2 - 1, body, 0)
    pair(n - 2, last=True)
    stage_c(n - 1, 1)

    oc = jnp.concatenate([oc_s[c] for c in range(hb * rep)], axis=1)
    acc_ref[...] += jax.lax.dot_general(
        wot_ref[j], oc, nt, preferred_element_type=jnp.float32)

    @pl.when(j == nj - 1)
    def _():
        for b in range(bb):
            o_ref[b] = acc_ref[:, b * sq:(b + 1) * sq].astype(o_ref.dtype)


@jax.jit
def pallas_standalone__gqa_block_cached__near_ridge_kernel(x, k_cache, v_cache, wq, wo):
    B, Sq, D = x.shape
    _, Hkv, Sk, Dh = k_cache.shape
    Hq = wq.shape[1] // Dh
    rep = Hq // Hkv
    hb, bb = HB, BB
    ng = Hkv // hb
    gw = hb * rep * Dh
    kern = functools.partial(_kernel, rep=rep, dh=Dh, hb=hb, bb=bb, ng=ng)
    R = rep * Sq
    out_t = pl.pallas_call(
        kern,
        grid=(B // bb, ng),
        in_specs=[
            pl.BlockSpec((bb, D, Sq), lambda b, j: (b, 0, 0)),
            pl.BlockSpec((bb, hb, Sk, Dh), lambda b, j: (b, j, 0, 0)),
            pl.BlockSpec((bb, hb, Sk, Dh), lambda b, j: (b, j, 0, 0)),
            pl.BlockSpec(memory_space=pl.ANY),
            pl.BlockSpec(memory_space=pl.ANY),
        ],
        out_specs=pl.BlockSpec((bb, D, Sq), lambda b, j: (b, 0, 0)),
        out_shape=jax.ShapeDtypeStruct((B, D, Sq), x.dtype),
        scratch_shapes=[pltpu.VMEM((ng, D, gw), jnp.bfloat16),
                        pltpu.VMEM((ng, D, gw), jnp.bfloat16),
                        pltpu.SemaphoreType.DMA((2, ng)),
                        pltpu.VMEM((D, bb * Sq), jnp.float32),
                        pltpu.VMEM((bb * Sq, D), jnp.bfloat16),
                        pltpu.VMEM((hb * bb, R, Dh), jnp.bfloat16),
                        pltpu.VMEM((hb * rep, bb * Sq, Dh), jnp.bfloat16),
                        pltpu.VMEM((R, Sk), jnp.float32),
                        pltpu.VMEM((R, Sk), jnp.float32),
                        pltpu.VMEM((R, Sk), jnp.bfloat16),
                        pltpu.VMEM((R, Sk), jnp.bfloat16),
                        pltpu.VMEM((R, 1), jnp.float32),
                        pltpu.VMEM((R, 1), jnp.float32)],
        compiler_params=pltpu.CompilerParams(
            dimension_semantics=("arbitrary", "arbitrary"),
            vmem_limit_bytes=100 * 1024 * 1024,
        ),
    )(x.transpose(0, 2, 1), k_cache, v_cache, wq, wo.T)
    return out_t.transpose(0, 2, 1)
```
